```python
import os as _os
_os.environ.setdefault("JAX_PLATFORMS", "cpu")
import jax
import jax.numpy as jnp

def _softmax(x, axis=-1):
    return jax.nn.softmax(x, axis=axis)
def _gelu(x):
    return jax.nn.gelu(x, approximate=True)
def _silu(x):
    return jax.nn.silu(x)
def _sigmoid(x):
    return jax.nn.sigmoid(x)
def _layernorm(x, axis=-1, eps=1e-5):
    m = jnp.mean(x, axis=axis, keepdims=True)
    v = jnp.var(x, axis=axis, keepdims=True)
    return (x - m) / jnp.sqrt(v + eps)
def _scatter_add(tgt, idx, src, axis=0):
    return tgt.at[idx].add(src)
def _segment_sum(src, seg, n):
    return jax.ops.segment_sum(src, seg, n)
class _Rng:
    def __init__(self, key):
        self._k = key
    def _next(self):
        self._k, sub = jax.random.split(self._k)
        return sub
    def normal(self, shape):
        return jax.random.normal(self._next(), shape, dtype=jnp.bfloat16)
    def randint(self, lo, hi, shape):
        return jax.random.randint(self._next(), shape, lo, hi, dtype=jnp.int32)
    def uniform(self, shape, lo=0.0, hi=1.0):
        return jax.random.uniform(self._next(), shape, jnp.bfloat16, lo, hi)
    def permutation(self, n):
        return jax.random.permutation(self._next(), n)


kernel_name = 'interleave_layers__spectral_gfnet__dense_activation_gelu__prompt'

def setup_inputs():
    _rng = _Rng(jax.random.key(int.from_bytes(__import__("os").urandom(4), "little")))
    _w = (lambda a: (lambda t: t.astype(jnp.bfloat16) if jnp.issubdtype(t.dtype, jnp.floating) else t)(jnp.asarray(a)))
    def _A_setup():
        B, S, D = 1, 2048, 640
        Df = D // 2 + 1
        return {
            "x": _w((lambda *s: _rng.normal(s) * 0.05)(B, S, D)),
            "w_r": _w((lambda *s: _rng.normal(s) * 0.2)(S, Df) * 0.02),
            "w_i": _w((lambda *s: _rng.normal(s) * 0.2)(S, Df) * 0.02),
        }
    _A_in = _A_setup()

    def _B_setup():
        B, S, D, F = 1, 2048, 640, 1728
        return {
            "x": _w((lambda *s: _rng.normal(s) * 0.05)(B, S, D)),
            "w1": _w((lambda *s: _rng.normal(s) * 0.1)(D, F) * (D ** -0.5)),
            "b1": _w((lambda *s: _rng.normal(s) * 0.1)(F) * 0.01),
            "w2": _w((lambda *s: _rng.normal(s) * 0.1)(F, D) * (F ** -0.5)),
            "b2": _w((lambda *s: _rng.normal(s) * 0.1)(D) * 0.01),
        }
    _B_in = _B_setup()

    return {
        "A_x": _A_in["x"],
        "A_w_r": _A_in["w_r"],
        "A_w_i": _A_in["w_i"],
        "B_x": _B_in["x"],
        "B_w1": _B_in["w1"],
        "B_b1": _B_in["b1"],
        "B_w2": _B_in["w2"],
        "B_b2": _B_in["b2"],
    }

def reference(A_x, A_w_r, A_w_i, B_x, B_w1, B_b1, B_w2, B_b2):
    def _A_ref(x, w_r, w_i):
        B, S, D = x.shape
        X = (lambda x, axes=(-2,-1): jnp.fft.rfft2(x.astype(jnp.float32), axes=axes))(x, axes=(-2, -1))
        W = w_r + 1j * w_i
        X = X * W
        y = (lambda x, s, axes=(-2,-1): jnp.fft.irfft2(x, s=s, axes=axes).astype(jnp.bfloat16))(X, (S, D), axes=(-2, -1))
        return y

    def _B_ref(x, w1, b1, w2, b2):
        h = jnp.einsum("bsd,df->bsf", x, w1) + b1
        h = _gelu(h)
        return jnp.einsum("bsf,fd->bsd", h, w2) + b2

    x = A_x
    x = x + _A_ref(_layernorm(x, axis=-1), A_w_r, A_w_i)
    x = x + _B_ref(_layernorm(x, axis=-1), B_w1, B_b1, B_w2, B_b2)
    x = x + _A_ref(_layernorm(x, axis=-1), A_w_r, A_w_i)
    x = x + _B_ref(_layernorm(x, axis=-1), B_w1, B_b1, B_w2, B_b2)
    return x
```

```python
import math

import jax
import jax.numpy as jnp
from jax import lax
import jax.experimental.pallas as pl
import jax.experimental.pallas.tpu as pltpu

S = 2048
D = 640
DF = D // 2 + 1
DP = 384
F = 1728
R = 16
M = S // R

_BF = jnp.bfloat16
_F32 = jnp.float32


def _cmul_const(re, im, wr, wi):
    eps = 1e-12
    if abs(wi) < eps:
        if abs(wr - 1.0) < eps:
            return re, im
        if abs(wr + 1.0) < eps:
            return -re, -im
        return re * wr, im * wr
    if abs(wr) < eps:
        if abs(wi - 1.0) < eps:
            return -im, re
        if abs(wi + 1.0) < eps:
            return im, -re
        return -im * wi, re * wi
    if abs(abs(wr) - abs(wi)) < eps:
        c = abs(wr)
        sr = 1.0 if wr > 0 else -1.0
        si = 1.0 if wi > 0 else -1.0
        a = (re * sr - im * si) if False else None
        if sr > 0 and si > 0:
            nr, ni = re - im, re + im
        elif sr > 0 and si < 0:
            nr, ni = re + im, im - re
        elif sr < 0 and si > 0:
            nr, ni = -re - im, re - im
        else:
            nr, ni = im - re, -re - im
        return nr * c, ni * c
    return re * wr - im * wi, re * wi + im * wr


def _fft_list(xs, sign):
    n = len(xs)
    if n == 1:
        return xs
    ev = _fft_list(xs[0::2], sign)
    od = _fft_list(xs[1::2], sign)
    out = [None] * n
    for k in range(n // 2):
        ang = sign * 2.0 * math.pi * k / n
        tr, ti = _cmul_const(od[k][0], od[k][1], math.cos(ang), math.sin(ang))
        out[k] = (ev[k][0] + tr, ev[k][1] + ti)
        out[k + n // 2] = (ev[k][0] - tr, ev[k][1] - ti)
    return out


def _layernorm_bf16(x_bf):
    x = x_bf.astype(_F32)
    m = jnp.mean(x, axis=-1, keepdims=True)
    xc = x - m
    v = jnp.mean(xc * xc, axis=-1, keepdims=True)
    m_b = m.astype(_BF).astype(_F32)
    v_b = v.astype(_BF).astype(_F32)
    d = (x - m_b).astype(_BF).astype(_F32)
    s = jnp.sqrt((v_b + 1e-5).astype(_BF).astype(_F32)).astype(_BF).astype(_F32)
    return (d / s).astype(_BF)


def _gelu_tanh(x):
    c = math.sqrt(2.0 / math.pi)
    return 0.5 * x * (1.0 + jnp.tanh(c * (x + 0.044715 * (x * x * x))))


def _kernel(x_ref, wr_ref, wi_ref, w1_ref, b1_ref, w2_ref, b2_ref, o_ref,
            cd_ref, icd_ref, g_ref, h_ref, z_ref, zb_ref):
    dd = lax.broadcasted_iota(jnp.int32, (D, DP), 0)
    jj = lax.broadcasted_iota(jnp.int32, (D, DP), 1)
    ang = ((dd * jj) % D).astype(_F32) * (2.0 * math.pi / D)
    valid = jj < DF
    cd_ref[:, 0:DP] = jnp.where(valid, jnp.cos(ang), 0.0).astype(_BF)
    cd_ref[:, DP:2 * DP] = jnp.where(valid, -jnp.sin(ang), 0.0).astype(_BF)

    jj = lax.broadcasted_iota(jnp.int32, (DP, D), 0)
    dd = lax.broadcasted_iota(jnp.int32, (DP, D), 1)
    ang = ((dd * jj) % D).astype(_F32) * (2.0 * math.pi / D)
    cj = jnp.where((jj == 0) | (jj == D // 2), 1.0, 2.0)
    cj = jnp.where(jj < DF, cj, 0.0)
    icd_ref[0:DP, :] = (cj * jnp.cos(ang)).astype(_BF)
    icd_ref[DP:2 * DP, :] = (-cj * jnp.sin(ang)).astype(_BF)

    k1 = lax.broadcasted_iota(jnp.int32, (R, M, M), 0)
    rr = lax.broadcasted_iota(jnp.int32, (R, M, M), 1)
    cc = lax.broadcasted_iota(jnp.int32, (R, M, M), 2)
    ang = ((cc * (k1 + R * rr)) % S).astype(_F32) * (2.0 * math.pi / S)
    g_ref[:, 0:M, :] = jnp.cos(ang).astype(_BF)
    g_ref[:, M:2 * M, :] = (-jnp.sin(ang)).astype(_BF)
    ang = ((rr * (k1 + R * cc)) % S).astype(_F32) * (2.0 * math.pi / S)
    h_ref[:, 0:M, :] = jnp.cos(ang).astype(_BF)
    h_ref[:, M:2 * M, :] = jnp.sin(ang).astype(_BF)

    o_ref[...] = x_ref[...]
    scale = 1.0 / (S * D)
    RB = 256

    def layer(_, carry):
        def fwd_d(i, c):
            rows = pl.ds(pl.multiple_of(i * RB, RB), RB)
            u = _layernorm_bf16(o_ref[rows, :])
            z_ref[rows, :] = jnp.dot(u, cd_ref[...], preferred_element_type=_F32)
            return c
        lax.fori_loop(0, S // RB, fwd_d, 0)

        blocks = [(z_ref[n * M:(n + 1) * M, 0:DP], z_ref[n * M:(n + 1) * M, DP:2 * DP])
                  for n in range(R)]
        a = _fft_list(blocks, -1.0)
        for k in range(R):
            zb_ref[k * M:(k + 1) * M, 0:DP] = a[k][0].astype(_BF)
            zb_ref[k * M:(k + 1) * M, DP:2 * DP] = a[k][1].astype(_BF)

        def mid(k, c):
            rows = pl.ds(pl.multiple_of(k * M, M), M)
            pq = jnp.dot(g_ref[k], zb_ref[rows, :], preferred_element_type=_F32)
            xr = pq[0:M, 0:DP] - pq[M:2 * M, DP:2 * DP]
            xi = pq[0:M, DP:2 * DP] + pq[M:2 * M, 0:DP]
            wr = wr_ref[rows, :].astype(_F32) * scale
            wi = wi_ref[rows, :].astype(_F32) * scale
            yr = xr * wr - xi * wi
            yi = xr * wi + xi * wr
            y = jnp.concatenate([yr.astype(_BF), yi.astype(_BF)], axis=1)
            pq = jnp.dot(h_ref[k], y, preferred_element_type=_F32)
            z_ref[rows, 0:DP] = pq[0:M, 0:DP] - pq[M:2 * M, DP:2 * DP]
            z_ref[rows, DP:2 * DP] = pq[0:M, DP:2 * DP] + pq[M:2 * M, 0:DP]
            return c
        lax.fori_loop(0, R, mid, 0)

        blocks = [(z_ref[n * M:(n + 1) * M, 0:DP], z_ref[n * M:(n + 1) * M, DP:2 * DP])
                  for n in range(R)]
        a = _fft_list(blocks, 1.0)
        for k in range(R):
            zb_ref[k * M:(k + 1) * M, 0:DP] = a[k][0].astype(_BF)
            zb_ref[k * M:(k + 1) * M, DP:2 * DP] = a[k][1].astype(_BF)

        def ffn(i, c):
            rows = pl.ds(pl.multiple_of(i * RB, RB), RB)
            y = jnp.dot(zb_ref[rows, :], icd_ref[...], preferred_element_type=_F32)
            x1 = (o_ref[rows, :].astype(_F32) + y.astype(_BF).astype(_F32)).astype(_BF)
            u = _layernorm_bf16(x1)
            hh = jnp.dot(u, w1_ref[...], preferred_element_type=_F32).astype(_BF)
            hh = (hh.astype(_F32) + b1_ref[...].astype(_F32)).astype(_BF)
            hh = _gelu_tanh(hh.astype(_F32)).astype(_BF)
            oo = jnp.dot(hh, w2_ref[...], preferred_element_type=_F32).astype(_BF)
            oo = (oo.astype(_F32) + b2_ref[...].astype(_F32)).astype(_BF)
            o_ref[rows, :] = (x1.astype(_F32) + oo.astype(_F32)).astype(_BF)
            return c
        lax.fori_loop(0, S // RB, ffn, 0)
        return carry

    lax.fori_loop(0, 2, layer, 0)


@jax.jit
def pallas_interleave_layers__spectral_gfnet__dense_activation_gelu__prompt_kernel(
    A_x: jax.Array,
    A_w_r: jax.Array,
    A_w_i: jax.Array,
    B_x: jax.Array,
    B_w1: jax.Array,
    B_b1: jax.Array,
    B_w2: jax.Array,
    B_b2: jax.Array,
):
    x = A_x.reshape(S, D)

    def prep(w):
        w = jnp.pad(w, ((0, 0), (0, DP - DF)))
        return w.reshape(M, R, DP).transpose(1, 0, 2).reshape(S, DP)

    out = pl.pallas_call(
        _kernel,
        out_shape=jax.ShapeDtypeStruct((S, D), _BF),
        scratch_shapes=[
            pltpu.VMEM((D, 2 * DP), _BF),
            pltpu.VMEM((2 * DP, D), _BF),
            pltpu.VMEM((R, 2 * M, M), _BF),
            pltpu.VMEM((R, 2 * M, M), _BF),
            pltpu.VMEM((S, 2 * DP), _F32),
            pltpu.VMEM((S, 2 * DP), _BF),
        ],
        compiler_params=pltpu.CompilerParams(vmem_limit_bytes=100 * 1024 * 1024),
    )(x, prep(A_w_r), prep(A_w_i), B_w1, B_b1.reshape(1, F), B_w2, B_b2.reshape(1, D))
    return out.reshape(1, S, D)
```

```python
import math

import jax
import jax.numpy as jnp
from jax import lax
import jax.experimental.pallas as pl
import jax.experimental.pallas.tpu as pltpu

S = 2048
D = 640
DF = D // 2 + 1
DP = 384
F = 1728
R = 16
M = S // R

_BF = jnp.bfloat16
_F32 = jnp.float32


def _cmul_const(re, im, wr, wi):
    eps = 1e-12
    if abs(wi) < eps:
        if abs(wr - 1.0) < eps:
            return re, im
        if abs(wr + 1.0) < eps:
            return -re, -im
        return re * wr, im * wr
    if abs(wr) < eps:
        if abs(wi - 1.0) < eps:
            return -im, re
        if abs(wi + 1.0) < eps:
            return im, -re
        return -im * wi, re * wi
    if abs(abs(wr) - abs(wi)) < eps:
        c = abs(wr)
        sr = 1.0 if wr > 0 else -1.0
        si = 1.0 if wi > 0 else -1.0
        a = (re * sr - im * si) if False else None
        if sr > 0 and si > 0:
            nr, ni = re - im, re + im
        elif sr > 0 and si < 0:
            nr, ni = re + im, im - re
        elif sr < 0 and si > 0:
            nr, ni = -re - im, re - im
        else:
            nr, ni = im - re, -re - im
        return nr * c, ni * c
    return re * wr - im * wi, re * wi + im * wr


def _fft_list(xs, sign):
    n = len(xs)
    if n == 1:
        return xs
    ev = _fft_list(xs[0::2], sign)
    od = _fft_list(xs[1::2], sign)
    out = [None] * n
    for k in range(n // 2):
        ang = sign * 2.0 * math.pi * k / n
        tr, ti = _cmul_const(od[k][0], od[k][1], math.cos(ang), math.sin(ang))
        out[k] = (ev[k][0] + tr, ev[k][1] + ti)
        out[k + n // 2] = (ev[k][0] - tr, ev[k][1] - ti)
    return out


def _layernorm_bf16(x_bf):
    x = x_bf.astype(_F32)
    m = jnp.mean(x, axis=-1, keepdims=True)
    xc = x - m
    v = jnp.mean(xc * xc, axis=-1, keepdims=True)
    m_b = m.astype(_BF).astype(_F32)
    v_b = v.astype(_BF).astype(_F32)
    d = (x - m_b).astype(_BF).astype(_F32)
    s = jnp.sqrt((v_b + 1e-5).astype(_BF).astype(_F32)).astype(_BF).astype(_F32)
    return (d / s).astype(_BF)


def _gelu_tanh(x):
    c = math.sqrt(2.0 / math.pi)
    return 0.5 * x * (1.0 + jnp.tanh(c * (x + 0.044715 * (x * x * x))))


def _kernel(x_ref, wr_ref, wi_ref, w1_ref, b1_ref, w2_ref, b2_ref, o_ref,
            cd_ref, icd_ref, g_ref, h_ref, z_ref, zb_ref):
    dd = lax.broadcasted_iota(jnp.int32, (D, DP), 0)
    jj = lax.broadcasted_iota(jnp.int32, (D, DP), 1)
    ang = ((dd * jj) % D).astype(_F32) * (2.0 * math.pi / D)
    valid = jj < DF
    cd_ref[:, 0:DP] = jnp.where(valid, jnp.cos(ang), 0.0).astype(_BF)
    cd_ref[:, DP:2 * DP] = jnp.where(valid, -jnp.sin(ang), 0.0).astype(_BF)

    jj = lax.broadcasted_iota(jnp.int32, (DP, D), 0)
    dd = lax.broadcasted_iota(jnp.int32, (DP, D), 1)
    ang = ((dd * jj) % D).astype(_F32) * (2.0 * math.pi / D)
    cj = jnp.where((jj == 0) | (jj == D // 2), 1.0, 2.0)
    cj = jnp.where(jj < DF, cj, 0.0)
    icd_ref[0:DP, :] = (cj * jnp.cos(ang)).astype(_BF)
    icd_ref[DP:2 * DP, :] = (-cj * jnp.sin(ang)).astype(_BF)

    k1 = lax.broadcasted_iota(jnp.int32, (R, M, M), 0)
    rr = lax.broadcasted_iota(jnp.int32, (R, M, M), 1)
    cc = lax.broadcasted_iota(jnp.int32, (R, M, M), 2)
    ang = ((cc * (k1 + R * rr)) % S).astype(_F32) * (2.0 * math.pi / S)
    g_ref[:, 0:M, :] = jnp.cos(ang).astype(_BF)
    g_ref[:, M:2 * M, :] = (-jnp.sin(ang)).astype(_BF)
    ang = ((rr * (k1 + R * cc)) % S).astype(_F32) * (2.0 * math.pi / S)
    h_ref[:, 0:M, :] = jnp.cos(ang).astype(_BF)
    h_ref[:, M:2 * M, :] = jnp.sin(ang).astype(_BF)

    o_ref[...] = x_ref[...]
    scale = 1.0 / (S * D)
    RB = 512

    def layer(_, carry):
        def fwd_d(i, c):
            rows = pl.ds(pl.multiple_of(i * RB, RB), RB)
            u = _layernorm_bf16(o_ref[rows, :])
            z_ref[rows, :] = jnp.dot(u, cd_ref[...], preferred_element_type=_F32)
            return c
        lax.fori_loop(0, S // RB, fwd_d, 0)

        blocks = [(z_ref[n * M:(n + 1) * M, 0:DP], z_ref[n * M:(n + 1) * M, DP:2 * DP])
                  for n in range(R)]
        a = _fft_list(blocks, -1.0)
        for k in range(R):
            zb_ref[k * M:(k + 1) * M, 0:DP] = a[k][0].astype(_BF)
            zb_ref[k * M:(k + 1) * M, DP:2 * DP] = a[k][1].astype(_BF)

        for k in range(R):
            rows = slice(k * M, (k + 1) * M)
            pq = jnp.dot(g_ref[k], zb_ref[rows, :], preferred_element_type=_F32)
            xr = pq[0:M, 0:DP] - pq[M:2 * M, DP:2 * DP]
            xi = pq[0:M, DP:2 * DP] + pq[M:2 * M, 0:DP]
            wr = wr_ref[rows, :].astype(_F32) * scale
            wi = wi_ref[rows, :].astype(_F32) * scale
            zb_ref[rows, 0:DP] = (xr * wr - xi * wi).astype(_BF)
            zb_ref[rows, DP:2 * DP] = (xr * wi + xi * wr).astype(_BF)
        for k in range(R):
            rows = slice(k * M, (k + 1) * M)
            pq = jnp.dot(h_ref[k], zb_ref[rows, :], preferred_element_type=_F32)
            z_ref[rows, 0:DP] = pq[0:M, 0:DP] - pq[M:2 * M, DP:2 * DP]
            z_ref[rows, DP:2 * DP] = pq[0:M, DP:2 * DP] + pq[M:2 * M, 0:DP]

        blocks = [(z_ref[n * M:(n + 1) * M, 0:DP], z_ref[n * M:(n + 1) * M, DP:2 * DP])
                  for n in range(R)]
        a = _fft_list(blocks, 1.0)
        for k in range(R):
            zb_ref[k * M:(k + 1) * M, 0:DP] = a[k][0].astype(_BF)
            zb_ref[k * M:(k + 1) * M, DP:2 * DP] = a[k][1].astype(_BF)

        def ffn(i, c):
            rows = pl.ds(pl.multiple_of(i * RB, RB), RB)
            y = jnp.dot(zb_ref[rows, :], icd_ref[...], preferred_element_type=_F32)
            x1 = (o_ref[rows, :].astype(_F32) + y.astype(_BF).astype(_F32)).astype(_BF)
            u = _layernorm_bf16(x1)
            hh = jnp.dot(u, w1_ref[...], preferred_element_type=_F32).astype(_BF)
            hh = (hh.astype(_F32) + b1_ref[...].astype(_F32)).astype(_BF)
            hh = _gelu_tanh(hh.astype(_F32)).astype(_BF)
            oo = jnp.dot(hh, w2_ref[...], preferred_element_type=_F32).astype(_BF)
            oo = (oo.astype(_F32) + b2_ref[...].astype(_F32)).astype(_BF)
            o_ref[rows, :] = (x1.astype(_F32) + oo.astype(_F32)).astype(_BF)
            return c
        lax.fori_loop(0, S // RB, ffn, 0)
        return carry

    lax.fori_loop(0, 2, layer, 0)


@jax.jit
def pallas_interleave_layers__spectral_gfnet__dense_activation_gelu__prompt_kernel(
    A_x: jax.Array,
    A_w_r: jax.Array,
    A_w_i: jax.Array,
    B_x: jax.Array,
    B_w1: jax.Array,
    B_b1: jax.Array,
    B_w2: jax.Array,
    B_b2: jax.Array,
):
    x = A_x.reshape(S, D)

    def prep(w):
        w = jnp.pad(w, ((0, 0), (0, DP - DF)))
        return w.reshape(M, R, DP).transpose(1, 0, 2).reshape(S, DP)

    out = pl.pallas_call(
        _kernel,
        out_shape=jax.ShapeDtypeStruct((S, D), _BF),
        scratch_shapes=[
            pltpu.VMEM((D, 2 * DP), _BF),
            pltpu.VMEM((2 * DP, D), _BF),
            pltpu.VMEM((R, 2 * M, M), _BF),
            pltpu.VMEM((R, 2 * M, M), _BF),
            pltpu.VMEM((S, 2 * DP), _F32),
            pltpu.VMEM((S, 2 * DP), _BF),
        ],
        compiler_params=pltpu.CompilerParams(vmem_limit_bytes=100 * 1024 * 1024),
    )(x, prep(A_w_r), prep(A_w_i), B_w1, B_b1.reshape(1, F), B_w2, B_b2.reshape(1, D))
    return out.reshape(1, S, D)
```
